```python
import jax
import jax.numpy as jnp

def _softmax(x, axis=-1):
    return jax.nn.softmax(x, axis=axis)
def _gelu(x):
    return jax.nn.gelu(x, approximate=True)
def _silu(x):
    return jax.nn.silu(x)
def _sigmoid(x):
    return jax.nn.sigmoid(x)
def _layernorm(x, axis=-1, eps=1e-5):
    m = jnp.mean(x, axis=axis, keepdims=True)
    v = jnp.var(x, axis=axis, keepdims=True)
    return (x - m) / jnp.sqrt(v + eps)
def _scatter_add(tgt, idx, src, axis=0):
    return tgt.at[idx].add(src)
def _segment_sum(src, seg, n):
    return jax.ops.segment_sum(src, seg, n)
class _Rng:
    def __init__(self, key):
        self._k = key
    def _next(self):
        self._k, sub = jax.random.split(self._k)
        return sub
    def normal(self, shape):
        return jax.random.normal(self._next(), shape, dtype=jnp.bfloat16)
    def randint(self, lo, hi, shape):
        return jax.random.randint(self._next(), shape, lo, hi, dtype=jnp.int32)
    def uniform(self, shape, lo=0.0, hi=1.0):
        return jax.random.uniform(self._next(), shape, jnp.bfloat16, lo, hi)
    def permutation(self, n):
        return jax.random.permutation(self._next(), n)


kernel_name = 'gated_mix__compressed_kv_cla__sliding_local_dilated__prompt'

def setup_inputs():
    _rng = _Rng(jax.random.key(int.from_bytes(__import__("os").urandom(4), "little")))
    _w = (lambda a: (lambda t: t.astype(jnp.bfloat16) if jnp.issubdtype(t.dtype, jnp.floating) else t)(jnp.asarray(a)))
    def _A_setup():
        B, H, Sq, Sk, D, M = 1, 32, 2048, 2048, 128, 1024
        Dc = 4 * D
        return {
            "x": _w((lambda *s: _rng.normal(s) * 0.05)(B, Sq, M)),
            "c_kv": _w((lambda *s: _rng.normal(s) * 0.05)(B, Sk, Dc)),
            "w_q": _w((lambda *s: _rng.normal(s) * 0.05)(M, H, D) * (M ** -0.5)),
            "w_uk": _w((lambda *s: _rng.normal(s) * 0.05)(Dc, H, D) * (Dc ** -0.5)),
            "w_uv": _w((lambda *s: _rng.normal(s) * 0.05)(Dc, H, D) * (Dc ** -0.5)),
            "w_o": _w((lambda *s: _rng.normal(s) * 0.05)(H, D, M) * ((H * D) ** -0.5)),
        }
    _A_in = _A_setup()

    def _B_setup():
        B, S, D = 1, 2048, 1024
        return {
            "x": _w((lambda *s: _rng.normal(s) * 0.05)(B, S, D)),
            "wqkv": _w((lambda *s: _rng.normal(s) * 0.05)(D, 3 * D)),
            "wo": _w((lambda *s: _rng.normal(s) * 0.05)(D, D)),
        }
    _B_in = _B_setup()

    return {
        "A_x": _A_in["x"],
        "A_c_kv": _A_in["c_kv"],
        "A_w_q": _A_in["w_q"],
        "A_w_uk": _A_in["w_uk"],
        "A_w_uv": _A_in["w_uv"],
        "A_w_o": _A_in["w_o"],
        "B_x": _B_in["x"],
        "B_wqkv": _B_in["wqkv"],
        "B_wo": _B_in["wo"],
        "gate_w": _w((lambda *s: _rng.normal(s) * 0.05)(1024)),
    }

def reference(A_x, A_c_kv, A_w_q, A_w_uk, A_w_uv, A_w_o, B_x, B_wqkv, B_wo, gate_w):
    def _A_ref(x, c_kv, w_q, w_uk, w_uv, w_o):
        B, Sq, M = x.shape[0], x.shape[1], x.shape[2]
        Sk = c_kv.shape[1]
        H, D = w_q.shape[1], w_q.shape[2]
        q = jnp.einsum("bqm,mhd->bhqd", x, w_q)
        k = jnp.einsum("bkc,chd->bhkd", c_kv, w_uk)
        v = jnp.einsum("bkc,chd->bhkd", c_kv, w_uv)
        scores = jnp.einsum("bhqd,bhkd->bhqk", q, k) * (D ** -0.5)
        off = Sk - Sq
        qi = jnp.arange(Sq)[:, None]
        kj = jnp.arange(Sk)[None, :]
        cmask = kj <= (qi + off)
        scores = jnp.where(cmask[None, None], scores, -1e9)
        p = _softmax(scores, axis=-1)
        ctx = jnp.einsum("bhqk,bhkd->bhqd", p, v)
        return jnp.einsum("bhqd,hdm->bqm", ctx, w_o)

    def _B_ref(x, wqkv, wo):
        B, S, D = x.shape
        H = 32; Dh = D // H
        W, dil = 8, 2
        qkv = (lambda x, *d: x.transpose(*d))((x @ wqkv).reshape(B, S, 3, H, Dh), 2, 0, 3, 1, 4)
        q, k, v = qkv[0], qkv[1], qkv[2]
        scale = Dh ** -0.5
        pos = jnp.arange(S)
        off = jnp.arange(W) * dil
        idx = pos[:, None] - off[None, :]
        mask = idx >= 0
        idx_c = jnp.where(mask, idx, 0).reshape(-1)
        kg = k[:, :, idx_c, :].reshape(B, H, S, W, Dh)
        vg = v[:, :, idx_c, :].reshape(B, H, S, W, Dh)
        logits = jnp.einsum("bhsd,bhswd->bhsw", q, kg) * scale
        logits = jnp.where(mask[None, None, :, :], logits, -1e9)
        attn = _softmax(logits, axis=-1)
        o = jnp.einsum("bhsw,bhswd->bhsd", attn, vg)
        return (lambda x, *d: x.transpose(*d))(o, 0, 2, 1, 3).reshape(B, S, D) @ wo

    x = A_x
    g = _sigmoid((x * gate_w).sum(-1, keepdims=True))
    a = _A_ref(x, A_c_kv, A_w_q, A_w_uk, A_w_uv, A_w_o)
    b = _B_ref(x, B_wqkv, B_wo)
    return g * a + (1 - g) * b
```

```python
import functools
import numpy as np
import jax
import jax.numpy as jnp
from jax import lax
import jax.experimental.pallas as pl
import jax.experimental.pallas.tpu as pltpu

S = 2048; M = 1024; H = 32; D = 128; DC = 512
LOG2E = 1.4426950408889634
F32 = jnp.float32; BF16 = jnp.bfloat16
NT = (((1,), (1,)), ((), ()))
PAD = 16
RB = 256
QB = 512
RF = 512


def _dot(a, b):
    return jnp.dot(a, b, preferred_element_type=F32)


def _kernel(x_hbm, c_hbm, wq_hbm, wk_hbm, wv_hbm, wo_hbm, wqkv_hbm, bwo_hbm, gw_ref,
            o_hbm,
            x_s, c_s, wq_s, wk_s, wv_s, wo_s, wqkv_s, ctx_s, g_s, kb_s, vb_s,
            w2q_s, w2k_s, w2v_s, q_s, kt_s, v_s, s_s, o_s, sems, osems):
    cps = [
        pltpu.make_async_copy(x_hbm, x_s, sems.at[0]),
        pltpu.make_async_copy(wqkv_hbm, wqkv_s, sems.at[1]),
        pltpu.make_async_copy(c_hbm, c_s, sems.at[2]),
        pltpu.make_async_copy(wq_hbm.bitcast(jnp.int32), wq_s, sems.at[3]),
        pltpu.make_async_copy(wk_hbm.bitcast(jnp.int32), wk_s, sems.at[4]),
        pltpu.make_async_copy(wv_hbm.bitcast(jnp.int32), wv_s, sems.at[5]),
        pltpu.make_async_copy(wo_hbm, wo_s.at[pl.ds(0, H * D), :], sems.at[6]),
        pltpu.make_async_copy(bwo_hbm, wo_s.at[pl.ds(H * D, M), :], sems.at[7]),
    ]
    for cp in cps:
        cp.start()
    cps[0].wait()
    with jax.named_scope("gate"):
        gw = gw_ref[...].astype(F32)
        for r in range(S // RB):
            xr = x_s[pl.ds(r * RB, RB), :].astype(F32)
            z = jnp.sum(xr * gw, axis=-1, keepdims=True)
            g = 1.0 / (1.0 + jnp.exp(-z))
            g_s[pl.ds(r * RB, RB), :] = jnp.broadcast_to(g, (RB, 128))
    cps[1].wait()
    zpad = jnp.zeros((PAD, M), F32)
    kb_s[pl.ds(0, PAD), :] = zpad
    vb_s[pl.ds(0, PAD), :] = zpad
    ri = lax.broadcasted_iota(jnp.int32, (128, 128), 0) // 32
    ci = lax.broadcasted_iota(jnp.int32, (128, 128), 1) // 32
    bd = jnp.where(ri == ci, 1.0, 0.0).astype(BF16)
    sc_b = (32 ** -0.5) * LOG2E

    def b_body(i, carry):
        r0 = pl.multiple_of(i * RB, RB)
        xr = x_s[pl.ds(r0, RB), :]
        kb_s.at[pl.ds(r0, RB + PAD), :][pl.ds(PAD, RB), :] = _dot(xr, wqkv_s[:, M:2 * M])
        vb_s.at[pl.ds(r0, RB + PAD), :][pl.ds(PAD, RB), :] = _dot(xr, wqkv_s[:, 2 * M:3 * M])
        q = _dot(xr, wqkv_s[:, 0:M]) * sc_b
        rows = r0 + lax.broadcasted_iota(jnp.int32, (RB, 128), 0)
        omg = 1.0 - g_s[pl.ds(r0, RB), :]
        kw = kb_s.at[pl.ds(r0, RB + PAD), :]
        vw = vb_s.at[pl.ds(r0, RB + PAD), :]
        for gi in range(M // 128):
            cs = slice(gi * 128, (gi + 1) * 128)
            qg = q[:, cs]
            lhs = jnp.concatenate(
                [(qg * kw[pl.ds(PAD - 2 * w, RB), cs]).astype(BF16) for w in range(8)], axis=0)
            lg = _dot(lhs, bd)
            lgs = [lg[0:RB]] + [jnp.where(rows >= 2 * w, lg[w * RB:(w + 1) * RB], -1e9) for w in range(1, 8)]
            m = lgs[0]
            for w in range(1, 8):
                m = jnp.maximum(m, lgs[w])
            den = None
            acc = None
            for w in range(8):
                e = jnp.exp2(lgs[w] - m)
                t = e * vw[pl.ds(PAD - 2 * w, RB), cs]
                den = e if den is None else den + e
                acc = t if acc is None else acc + t
            ctx_s[pl.ds(r0, RB), H * D + gi * 128:H * D + (gi + 1) * 128] = (acc * (omg / den)).astype(BF16)
        return carry

    with jax.named_scope("bbranch"):
        lax.fori_loop(0, S // RB, b_body, 0)

    for j in (2, 3, 4, 5):
        cps[j].wait()

    sc_a = (D ** -0.5) * LOG2E
    tri = (lax.broadcasted_iota(jnp.int32, (128, 128), 1)
           <= lax.broadcasted_iota(jnp.int32, (128, 128), 0))

    def gather(src, n, hp, dst):
        words = src[pl.ds(hp, n, stride=16), :]
        dst[:, 0:128] = pltpu.bitcast(words << 16, F32).astype(BF16)
        dst[:, 128:256] = pltpu.bitcast(words & jnp.int32(-65536), F32).astype(BF16)

    def attend(hh, hcol):
        cs = slice(hh * 128, (hh + 1) * 128)
        for qb in range(S // QB):
            r0 = qb * QB
            nsub = QB // 128
            mx = None
            for j in range((qb + 1) * nsub):
                a = max(0, j - qb * nsub)
                qv = q_s[pl.ds(r0 + a * 128, QB - a * 128), cs]
                st = _dot(qv, kt_s[cs, pl.ds(j * 128, 128)])
                if j >= qb * nsub:
                    top = jnp.where(tri, st[0:128], -1e9)
                    st = top if a == nsub - 1 else jnp.concatenate([top, st[128:]], axis=0)
                s_s[pl.ds(a * 128, QB - a * 128), pl.ds(j * 128, 128)] = st
                if mx is None:
                    mx = st
                elif a == 0:
                    mx = jnp.maximum(mx, st)
                else:
                    mx = jnp.concatenate([mx[0:a * 128], jnp.maximum(mx[a * 128:], st)], axis=0)
            m = jnp.broadcast_to(jnp.max(mx, axis=1, keepdims=True), (QB, 128))
            lacc = None
            acc = None
            for j in range((qb + 1) * nsub):
                a = max(0, j - qb * nsub)
                p = jnp.exp2(s_s[pl.ds(a * 128, QB - a * 128), pl.ds(j * 128, 128)] - m[a * 128:])
                pv = _dot(p.astype(BF16), v_s[pl.ds(j * 128, 128), cs])
                if acc is None:
                    lacc, acc = p, pv
                elif a == 0:
                    lacc, acc = lacc + p, acc + pv
                else:
                    lacc = jnp.concatenate([lacc[0:a * 128], lacc[a * 128:] + p], axis=0)
                    acc = jnp.concatenate([acc[0:a * 128], acc[a * 128:] + pv], axis=0)
            l = jnp.sum(lacc, axis=1, keepdims=True)
            ctx_s[pl.ds(r0, QB), pl.ds(hcol, 128)] = (acc * (g_s[pl.ds(r0, QB), :] / l)).astype(BF16)

    def a_body(hp, carry):
        with jax.named_scope("proj"):
            gather(wq_s, M, hp, w2q_s)
            gather(wk_s, DC, hp, w2k_s)
            gather(wv_s, DC, hp, w2v_s)
            q_s[...] = (_dot(x_s[...], w2q_s[...]) * sc_a).astype(BF16)
            kt_s[...] = _dot(c_s[...], w2k_s[...]).astype(BF16).T
            v_s[...] = _dot(c_s[...], w2v_s[...]).astype(BF16)
        with jax.named_scope("attn"):
            for hh in range(2):
                attend(hh, pl.multiple_of(hp * 256 + hh * 128, 128))
        return carry

    with jax.named_scope("abranch"):
        lax.fori_loop(0, H // 2, a_body, 0)

    cps[6].wait()
    cps[7].wait()
    with jax.named_scope("final"):
        ocps = []
        for r in range(S // RF):
            o_s[pl.ds(r * RF, RF), :] = _dot(ctx_s[pl.ds(r * RF, RF), :], wo_s[...]).astype(BF16)
            cp = pltpu.make_async_copy(o_s.at[pl.ds(r * RF, RF), :], o_hbm.at[pl.ds(r * RF, RF), :], osems.at[r])
            cp.start()
            ocps.append(cp)
        for cp in ocps:
            cp.wait()


@jax.jit
def pallas_gated_mix__compressed_kv_cla__sliding_local_dilated__prompt_kernel(
    A_x, A_c_kv, A_w_q, A_w_uk, A_w_uv, A_w_o, B_x, B_wqkv, B_wo, gate_w):
    del B_x
    any_spec = pl.BlockSpec(memory_space=pl.ANY)
    out = pl.pallas_call(
        _kernel,
        out_shape=jax.ShapeDtypeStruct((S, M), BF16),
        in_specs=[any_spec] * 8 + [pl.BlockSpec(memory_space=pltpu.VMEM)],
        out_specs=any_spec,
        scratch_shapes=[
            pltpu.VMEM((S, M), BF16),
            pltpu.VMEM((S, DC), BF16),
            pltpu.VMEM((M * 16, 128), jnp.int32),
            pltpu.VMEM((DC * 16, 128), jnp.int32),
            pltpu.VMEM((DC * 16, 128), jnp.int32),
            pltpu.VMEM((H * D + M, M), BF16),
            pltpu.VMEM((M, 3 * M), BF16),
            pltpu.VMEM((S, H * D + M), BF16),
            pltpu.VMEM((S, 128), F32),
            pltpu.VMEM((PAD + S, M), F32),
            pltpu.VMEM((PAD + S, M), F32),
            pltpu.VMEM((M, 256), BF16),
            pltpu.VMEM((DC, 256), BF16),
            pltpu.VMEM((DC, 256), BF16),
            pltpu.VMEM((S, 256), BF16),
            pltpu.VMEM((256, S), BF16),
            pltpu.VMEM((S, 256), BF16),
            pltpu.VMEM((QB, S), F32),
            pltpu.VMEM((S, M), BF16),
            pltpu.SemaphoreType.DMA((8,)),
            pltpu.SemaphoreType.DMA((S // RF,)),
        ],
        compiler_params=pltpu.CompilerParams(vmem_limit_bytes=120 * 1024 * 1024),
    )(A_x.reshape(S, M), A_c_kv.reshape(S, DC), A_w_q.reshape(M * H, D), A_w_uk.reshape(DC * H, D),
      A_w_uv.reshape(DC * H, D), A_w_o.reshape(H * D, M), B_wqkv, B_wo, gate_w.reshape(1, M))
    return out.reshape(1, S, M)
```

```python
import functools
import numpy as np
import jax
import jax.numpy as jnp
from jax import lax
import jax.experimental.pallas as pl
import jax.experimental.pallas.tpu as pltpu

S = 2048; M = 1024; H = 32; D = 128; DC = 512
LOG2E = 1.4426950408889634
F32 = jnp.float32; BF16 = jnp.bfloat16
NT = (((1,), (1,)), ((), ()))
PAD = 16
BS = 8
RB = 512
QB = 512
SOFF = [QB * (i * (i + 1) // 2) for i in range(S // QB + 1)]
TIE = False
PLAN = [(0,0),(0,1),(0,2),(0,3),'qk',(1,0),(1,1),(1,2),(1,3),'v']
RF = 256


def _rcp(x):
    r = pl.reciprocal(x, approx=True)
    return r * (2.0 - x * r)


def _dot(a, b):
    return jnp.dot(a, b, preferred_element_type=F32)


def _kernel(x_hbm, c_hbm, wq_hbm, wk_hbm, wv_hbm, wo_hbm, wqkv_hbm, bwo_hbm, gw_ref,
            o_hbm,
            x_s, c_s, wq_s, wk_s, wv_s, wo_s, ctx_s, g_s,
            w2q_s, w2k_s, w2v_s, q0_s, kt0_s, v0_s, q1_s, kt1_s, v1_s, sems, osems):
    o_s = x_s
    NXC = S // RB
    GSETS = ((0, 1), (1, 3), (3, M // 128))
    cps = [
        pltpu.make_async_copy(c_hbm, c_s, sems.at[0]),
        pltpu.make_async_copy(wq_hbm.bitcast(jnp.int32), wq_s, sems.at[1]),
        pltpu.make_async_copy(wk_hbm.bitcast(jnp.int32), wk_s, sems.at[2]),
        pltpu.make_async_copy(wv_hbm.bitcast(jnp.int32), wv_s, sems.at[3]),
        pltpu.make_async_copy(wo_hbm, wo_s.at[pl.ds(0, H * D), :], sems.at[4]),
        pltpu.make_async_copy(bwo_hbm, wo_s.at[pl.ds(H * D, M), :], sems.at[5]),
    ]

    def b_phase(wqkv_s, kb_s, vb_s, qb_s):
        xcp = [pltpu.make_async_copy(x_hbm.at[pl.ds(i * RB, RB), :], x_s.at[pl.ds(i * RB, RB), :], sems.at[6 + i])
               for i in range(NXC)]
        wcp = []
        for n, (g0, g1) in enumerate(GSETS):
            wcp.append([pltpu.make_async_copy(
                wqkv_hbm.at[:, pl.ds(p * M + g0 * 128, (g1 - g0) * 128)],
                wqkv_s.at[:, pl.ds(p * M + g0 * 128, (g1 - g0) * 128)], sems.at[6 + NXC + n])
                for p in (1, 2, 0)])
        xcp[0].start()
        for cp in wcp[0]:
            cp.start()
        gw = gw_ref[...].astype(F32)

        def arrive(i, g):
            if g == 0:
                xcp[i].wait()
                for r in range(RB // 256):
                    rows = pl.ds(i * RB + r * 256, 256)
                    zg = jnp.sum(x_s[rows, :].astype(F32) * gw, axis=-1, keepdims=True)
                    g_s[rows, :] = jnp.broadcast_to(1.0 / (1.0 + jnp.exp(-zg)), (256, 128))
                if i == 1:
                    for cp in cps:
                        cp.start()
            if i == 0:
                for n, (g0, g1) in enumerate(GSETS):
                    if g == g0:
                        for cp in wcp[n]:
                            cp.wait()
                        if n + 1 < len(GSETS):
                            for cp in wcp[n + 1]:
                                cp.start()
                        else:
                            for cp in xcp[1:]:
                                cp.start()

        zpad = jnp.zeros((PAD, M), F32)
        kb_s[pl.ds(0, PAD), :] = zpad
        vb_s[pl.ds(0, PAD), :] = zpad
        ri = lax.broadcasted_iota(jnp.int32, (128, 128), 0) // 32
        ci = lax.broadcasted_iota(jnp.int32, (128, 128), 1) // 32
        bd = jnp.where(ri == ci, 1.0, 0.0).astype(BF16)
        sc_b = (32 ** -0.5) * LOG2E

        NG = M // 128
        slots = [(i, g) for i in range(S // RB) for g in range(NG)]

        def b_proj(i, g):
            arrive(i, g)
            r0 = i * RB
            xr = x_s[pl.ds(r0, RB), :]
            c0 = g * 128
            kb_s[pl.ds(PAD + r0, RB), pl.ds(c0, 128)] = _dot(xr, wqkv_s[:, pl.ds(M + c0, 128)])
            vb_s[pl.ds(PAD + r0, RB), pl.ds(c0, 128)] = _dot(xr, wqkv_s[:, pl.ds(2 * M + c0, 128)])
            qb_s[(i * NG + g) % 2] = _dot(xr, wqkv_s[:, pl.ds(c0, 128)]) * sc_b

        def b_attn(i, g):
            r0 = i * RB
            cs = pl.ds(g * 128, 128)
            q = qb_s.at[(i * NG + g) % 2]
            pieces = []
            for t in range(RB // BS):
                t0 = r0 + t * BS
                qv = q[pl.ds(t * BS, BS), :]
                for j in range(4):
                    kk = kb_s[pl.ds(PAD + t0 - 8 - 2 * j, BS + 8), cs]
                    pieces.append((qv * kk[8:]).astype(BF16))
                    pieces.append((qv * kk[:BS]).astype(BF16))
            lg = _dot(jnp.concatenate(pieces, axis=0), bd)
            ws = [0, 4, 1, 5, 2, 6, 3, 7]
            for t in range(RB // BS):
                t0 = r0 + t * BS
                lgs = [lg[(t * 8 + n) * BS:(t * 8 + n + 1) * BS] for n in range(8)]
                if t0 < 14:
                    rows = t0 + lax.broadcasted_iota(jnp.int32, (BS, 128), 0)
                    lgs = [lgs[0]] + [jnp.where(rows >= 2 * ws[n], lgs[n], -1e9) for n in range(1, 8)]
                m = lgs[0]
                for n in range(1, 8):
                    m = jnp.maximum(m, lgs[n])
                den = None
                acc = None
                for j in range(4):
                    vv = vb_s[pl.ds(PAD + t0 - 8 - 2 * j, BS + 8), cs]
                    e0 = jnp.exp2(lgs[2 * j] - m)
                    e1 = jnp.exp2(lgs[2 * j + 1] - m)
                    d = e0 + e1
                    a = e0 * vv[8:] + e1 * vv[:BS]
                    den = d if den is None else den + d
                    acc = a if acc is None else acc + a
                omg = 1.0 - g_s[pl.ds(t0, BS), :]
                ctx_s[pl.ds(t0, BS), pl.ds(H * D + g * 128, 128)] = (acc * (omg * _rcp(den))).astype(BF16)

        with jax.named_scope("bbranch"):
            b_proj(*slots[0])
            for n, sl in enumerate(slots):
                if n + 1 < len(slots):
                    b_proj(*slots[n + 1])
                b_attn(*sl)

    pl.run_scoped(b_phase, pltpu.VMEM((M, 3 * M), BF16), pltpu.VMEM((PAD + S, M), F32), pltpu.VMEM((PAD + S, M), F32),
                  pltpu.VMEM((2, RB, 128), F32))

    def a_phase(s_s):
        for j in (0, 1, 2, 3):
            cps[j].wait()

        sc_a = (D ** -0.5) * LOG2E
        tri = (lax.broadcasted_iota(jnp.int32, (128, 128), 1)
               <= lax.broadcasted_iota(jnp.int32, (128, 128), 0))

        def gather(src, n, hp, dst):
            words = src[pl.ds(hp, n, stride=16), :]
            dst[:, 0:128] = pltpu.bitcast(words << 16, F32).astype(BF16)
            dst[:, 128:256] = pltpu.bitcast(words & jnp.int32(-65536), F32).astype(BF16)

        def tmax(t):
            n = t.shape[1] // 128
            parts = [t[:, i * 128:(i + 1) * 128] for i in range(n)]
            while len(parts) > 1:
                parts = [jnp.maximum(parts[i], parts[i + 1]) if i + 1 < len(parts) else parts[i]
                         for i in range(0, len(parts), 2)]
            return parts[0]

        def tsum(t):
            n = t.shape[1] // 128
            parts = [t[:, i * 128:(i + 1) * 128] for i in range(n)]
            while len(parts) > 1:
                parts = [parts[i] + parts[i + 1] if i + 1 < len(parts) else parts[i]
                         for i in range(0, len(parts), 2)]
            return parts[0]

        def tie(p, lsum):
            n = p.shape[1] - 128
            last = jnp.minimum(p[:, n:], lsum)
            return last if n == 0 else jnp.concatenate([p[:, :n], last], axis=1)

        def attend(bufs, hh, hcol, qbs):
            q_s, kt_s, v_s = bufs
            cs = slice(hh * 128, (hh + 1) * 128)
            nsub = QB // 128
            for qb in qbs:
                r0 = qb * QB
                so = SOFF[qb]
                mx = None
                for c in range(qb):
                    st = _dot(q_s[pl.ds(r0, QB), cs], kt_s[cs, pl.ds(c * QB, QB)])
                    s_s[:, pl.ds(so + c * QB, QB)] = st
                    mx = tmax(st) if mx is None else jnp.maximum(mx, tmax(st))
                ms = []
                for a in range(nsub):
                    w = (a + 1) * 128
                    st = _dot(q_s[pl.ds(r0 + a * 128, 128), cs], kt_s[cs, pl.ds(r0, w)])
                    last = jnp.where(tri, st[:, a * 128:], -1e9)
                    st = last if a == 0 else jnp.concatenate([st[:, :a * 128], last], axis=1)
                    s_s[pl.ds(a * 128, 128), pl.ds(so + r0, w)] = st
                    ma = tmax(st)
                    if mx is not None:
                        ma = jnp.maximum(ma, mx[a * 128:(a + 1) * 128])
                    ms.append(jnp.broadcast_to(jnp.max(ma, axis=1, keepdims=True), (128, 128)))
                m = jnp.concatenate(ms, axis=0)
                lacc = None
                acc = None
                for c in range(qb):
                    p = jnp.exp2(s_s[:, pl.ds(so + c * QB, QB)] - jnp.concatenate([m] * nsub, axis=1))
                    lacc = tsum(p) if lacc is None else lacc + tsum(p)
                    pv = _dot((tie(p, lacc) if TIE else p).astype(BF16), v_s[pl.ds(c * QB, QB), cs])
                    acc = pv if acc is None else acc + pv
                for a in range(nsub):
                    w = (a + 1) * 128
                    p = jnp.exp2(s_s[pl.ds(a * 128, 128), pl.ds(so + r0, w)]
                                 - jnp.concatenate([ms[a]] * (a + 1), axis=1))
                    la = tsum(p)
                    if acc is not None:
                        la = la + lacc[a * 128:(a + 1) * 128]
                    pv = _dot((tie(p, la) if TIE else p).astype(BF16), v_s[pl.ds(r0, w), cs])
                    if acc is not None:
                        pv = pv + acc[a * 128:(a + 1) * 128]
                    l = jnp.broadcast_to(jnp.sum(la, axis=1, keepdims=True), (128, 128))
                    ctx_s[pl.ds(r0 + a * 128, 128), pl.ds(hcol, 128)] = (
                        pv * (g_s[pl.ds(r0 + a * 128, 128), :] * _rcp(l))).astype(BF16)

        def proj(hp, bufs, parts="qkv"):
            q_s, kt_s, v_s = bufs
            if "k" in parts:
                gather(wk_s, DC, hp, w2k_s)
                kt_s[...] = _dot(c_s[...], w2k_s[...]).astype(BF16).T
            if "q" in parts:
                gather(wq_s, M, hp, w2q_s)
                q_s[...] = (_dot(x_s[...], w2q_s[...]) * sc_a).astype(BF16)
            if "v" in parts:
                gather(wv_s, DC, hp, w2v_s)
                v_s[...] = _dot(c_s[...], w2v_s[...]).astype(BF16)

        def attn_proj(hp, bufs, hpn, bufsn):
            for item in PLAN:
                if isinstance(item, str):
                    proj(hpn, bufsn, item)
                else:
                    hh, qb = item
                    attend(bufs, hh, pl.multiple_of(hp * 256 + hh * 128, 128), [qb])

        buf = ((q0_s, kt0_s, v0_s), (q1_s, kt1_s, v1_s))
        proj(0, buf[0])

        def a_body(i, carry):
            attn_proj(2 * i, buf[0], 2 * i + 1, buf[1])
            attn_proj(2 * i + 1, buf[1], jnp.minimum(2 * i + 2, H // 2 - 1), buf[0])
            return carry

        with jax.named_scope("abranch"):
            lax.fori_loop(0, H // 4, a_body, 0)

    pl.run_scoped(a_phase, pltpu.VMEM((QB, SOFF[S // QB]), F32))

    cps[4].wait()
    cps[5].wait()
    with jax.named_scope("final"):
        ocps = []
        for r in range(S // RF):
            o_s[pl.ds(r * RF, RF), :] = _dot(ctx_s[pl.ds(r * RF, RF), :], wo_s[...]).astype(BF16)
            cp = pltpu.make_async_copy(o_s.at[pl.ds(r * RF, RF), :], o_hbm.at[pl.ds(r * RF, RF), :], osems.at[r])
            cp.start()
            ocps.append(cp)
        for cp in ocps:
            cp.wait()


@jax.jit
def pallas_gated_mix__compressed_kv_cla__sliding_local_dilated__prompt_kernel(
    A_x, A_c_kv, A_w_q, A_w_uk, A_w_uv, A_w_o, B_x, B_wqkv, B_wo, gate_w):
    del B_x
    any_spec = pl.BlockSpec(memory_space=pl.ANY)
    out = pl.pallas_call(
        _kernel,
        out_shape=jax.ShapeDtypeStruct((S, M), BF16),
        in_specs=[any_spec] * 8 + [pl.BlockSpec(memory_space=pltpu.VMEM)],
        out_specs=any_spec,
        scratch_shapes=[
            pltpu.VMEM((S, M), BF16),
            pltpu.VMEM((S, DC), BF16),
            pltpu.VMEM((M * 16, 128), jnp.int32),
            pltpu.VMEM((DC * 16, 128), jnp.int32),
            pltpu.VMEM((DC * 16, 128), jnp.int32),
            pltpu.VMEM((H * D + M, M), BF16),
            pltpu.VMEM((S, H * D + M), BF16),
            pltpu.VMEM((S, 128), F32),
            pltpu.VMEM((M, 256), BF16),
            pltpu.VMEM((DC, 256), BF16),
            pltpu.VMEM((DC, 256), BF16),
            pltpu.VMEM((S, 256), BF16),
            pltpu.VMEM((256, S), BF16),
            pltpu.VMEM((S, 256), BF16),
            pltpu.VMEM((S, 256), BF16),
            pltpu.VMEM((256, S), BF16),
            pltpu.VMEM((S, 256), BF16),
            pltpu.SemaphoreType.DMA((6 + S // RB + 3,)),
            pltpu.SemaphoreType.DMA((S // RF,)),
        ],
        compiler_params=pltpu.CompilerParams(vmem_limit_bytes=120 * 1024 * 1024),
    )(A_x.reshape(S, M), A_c_kv.reshape(S, DC), A_w_q.reshape(M * H, D), A_w_uk.reshape(DC * H, D),
      A_w_uv.reshape(DC * H, D), A_w_o.reshape(H * D, M), B_wqkv, B_wo, gate_w.reshape(1, M))
    return out.reshape(1, S, M)
```

```python
import jax
import jax.numpy as jnp
from jax import lax
import jax.experimental.pallas as pl
import jax.experimental.pallas.tpu as pltpu

S = 2048; M = 1024; H = 32; D = 128; DC = 512
LOG2E = 1.4426950408889634
F32 = jnp.float32; BF16 = jnp.bfloat16
PAD = 16
BS = 8
RB = 512
QB = 512
SOFF = [QB * (i * (i + 1) // 2) for i in range(S // QB + 1)]
PLAN = [(0,0),(0,1),(0,2),(0,3),'qk',(1,0),(1,1),(1,2),(1,3),'v']
RF = 128


def _rcp(x):
    r = pl.reciprocal(x, approx=True)
    return r * (2.0 - x * r)


def _dot(a, b):
    return jnp.dot(a, b, preferred_element_type=F32)


def _kernel(x_hbm, c_hbm, wq_hbm, wk_hbm, wv_hbm, wo_hbm, wqkv_hbm, bwo_hbm, gw_ref,
            o_hbm,
            x_s, c_s, wq_s, wk_s, wv_s, wo_s, ctx_s, g_s,
            w2q_s, w2k_s, w2v_s, q0_s, kt0_s, v0_s, q1_s, kt1_s, v1_s, sems, osems):
    o_s = x_s
    NXC = S // RB
    GSETS = ((0, 1), (1, 2), (2, 4), (4, M // 128))
    cps = [
        pltpu.make_async_copy(c_hbm, c_s, sems.at[0]),
        pltpu.make_async_copy(wq_hbm.bitcast(jnp.int32), wq_s, sems.at[1]),
        pltpu.make_async_copy(wk_hbm.bitcast(jnp.int32), wk_s, sems.at[2]),
        pltpu.make_async_copy(wv_hbm.bitcast(jnp.int32), wv_s, sems.at[3]),
        pltpu.make_async_copy(wo_hbm, wo_s.at[pl.ds(0, H * D), :], sems.at[4]),
        pltpu.make_async_copy(bwo_hbm, wo_s.at[pl.ds(H * D, M), :], sems.at[5]),
    ]

    def b_phase(wqkv_s, kb_s, vb_s, qb_s):
        xcp = [pltpu.make_async_copy(x_hbm.at[pl.ds(i * RB, RB), :], x_s.at[pl.ds(i * RB, RB), :], sems.at[6 + i])
               for i in range(NXC)]
        wcp = []
        for n, (g0, g1) in enumerate(GSETS):
            wcp.append([pltpu.make_async_copy(
                wqkv_hbm.at[:, pl.ds(p * M + g0 * 128, (g1 - g0) * 128)],
                wqkv_s.at[:, pl.ds(p * M + g0 * 128, (g1 - g0) * 128)], sems.at[6 + NXC + n])
                for p in (1, 2, 0)])
        xcp[0].start()
        for cp in wcp[0]:
            cp.start()
        gw = gw_ref[...].astype(F32)

        def arrive(i, g):
            if g == 0:
                xcp[i].wait()
                for r in range(RB // 256):
                    rows = pl.ds(i * RB + r * 256, 256)
                    zg = jnp.sum(x_s[rows, :].astype(F32) * gw, axis=-1, keepdims=True)
                    g_s[rows, :] = jnp.broadcast_to(1.0 / (1.0 + jnp.exp(-zg)), (256, 128))
                if i == 1:
                    for cp in cps:
                        cp.start()
            if i == 0:
                for n, (g0, g1) in enumerate(GSETS):
                    if g == g0:
                        for cp in wcp[n]:
                            cp.wait()
                        if n + 1 < len(GSETS):
                            for cp in wcp[n + 1]:
                                cp.start()
                        else:
                            for cp in xcp[1:]:
                                cp.start()

        zpad = jnp.zeros((PAD, M), F32)
        kb_s[pl.ds(0, PAD), :] = zpad
        vb_s[pl.ds(0, PAD), :] = zpad
        ri = lax.broadcasted_iota(jnp.int32, (128, 128), 0) // 32
        ci = lax.broadcasted_iota(jnp.int32, (128, 128), 1) // 32
        bd = jnp.where(ri == ci, 1.0, 0.0).astype(BF16)
        sc_b = (32 ** -0.5) * LOG2E

        NG = M // 128
        slots = [(i, g) for i in range(S // RB) for g in range(NG)]

        def b_proj(i, g):
            arrive(i, g)
            r0 = i * RB
            xr = x_s[pl.ds(r0, RB), :]
            c0 = g * 128
            kb_s[pl.ds(PAD + r0, RB), pl.ds(c0, 128)] = _dot(xr, wqkv_s[:, pl.ds(M + c0, 128)])
            vb_s[pl.ds(PAD + r0, RB), pl.ds(c0, 128)] = _dot(xr, wqkv_s[:, pl.ds(2 * M + c0, 128)])
            qb_s[(i * NG + g) % 2] = _dot(xr, wqkv_s[:, pl.ds(c0, 128)]) * sc_b

        def b_attn(i, g):
            r0 = i * RB
            cs = pl.ds(g * 128, 128)
            q = qb_s.at[(i * NG + g) % 2]
            pieces = []
            for t in range(RB // BS):
                t0 = r0 + t * BS
                qv = q[pl.ds(t * BS, BS), :]
                for j in range(4):
                    kk = kb_s[pl.ds(PAD + t0 - 8 - 2 * j, BS + 8), cs]
                    pieces.append((qv * kk[8:]).astype(BF16))
                    pieces.append((qv * kk[:BS]).astype(BF16))
            lg = _dot(jnp.concatenate(pieces, axis=0), bd)
            ws = [0, 4, 1, 5, 2, 6, 3, 7]
            for t in range(RB // BS):
                t0 = r0 + t * BS
                lgs = [lg[(t * 8 + n) * BS:(t * 8 + n + 1) * BS] for n in range(8)]
                if t0 < 14:
                    rows = t0 + lax.broadcasted_iota(jnp.int32, (BS, 128), 0)
                    lgs = [lgs[0]] + [jnp.where(rows >= 2 * ws[n], lgs[n], -1e9) for n in range(1, 8)]
                m = lgs[0]
                for n in range(1, 8):
                    m = jnp.maximum(m, lgs[n])
                den = None
                acc = None
                for j in range(4):
                    vv = vb_s[pl.ds(PAD + t0 - 8 - 2 * j, BS + 8), cs]
                    e0 = jnp.exp2(lgs[2 * j] - m)
                    e1 = jnp.exp2(lgs[2 * j + 1] - m)
                    d = e0 + e1
                    a = e0 * vv[8:] + e1 * vv[:BS]
                    den = d if den is None else den + d
                    acc = a if acc is None else acc + a
                omg = 1.0 - g_s[pl.ds(t0, BS), :]
                ctx_s[pl.ds(t0, BS), pl.ds(H * D + g * 128, 128)] = (acc * (omg * _rcp(den))).astype(BF16)

        with jax.named_scope("bbranch"):
            b_proj(*slots[0])
            for n, sl in enumerate(slots):
                if n + 1 < len(slots):
                    b_proj(*slots[n + 1])
                b_attn(*sl)

    pl.run_scoped(b_phase, pltpu.VMEM((M, 3 * M), BF16), pltpu.VMEM((PAD + S, M), F32), pltpu.VMEM((PAD + S, M), F32),
                  pltpu.VMEM((2, RB, 128), F32))

    def final():
        ocps = []
        for r in range(S // RF):
            o_s[pl.ds(r * RF, RF), :] = _dot(ctx_s[pl.ds(r * RF, RF), :], wo_s[...]).astype(BF16)
            cp = pltpu.make_async_copy(o_s.at[pl.ds(r * RF, RF), :], o_hbm.at[pl.ds(r * RF, RF), :], osems.at[r])
            cp.start()
            ocps.append(cp)
        for cp in ocps:
            cp.wait()

    def a_phase(s_s):
        for j in (0, 1, 2, 3):
            cps[j].wait()

        sc_a = (D ** -0.5) * LOG2E
        tri = (lax.broadcasted_iota(jnp.int32, (128, 128), 1)
               <= lax.broadcasted_iota(jnp.int32, (128, 128), 0))

        def gather(src, n, hp, dst):
            words = src[pl.ds(hp, n, stride=16), :]
            dst[:, 0:128] = pltpu.bitcast(words << 16, F32).astype(BF16)
            dst[:, 128:256] = pltpu.bitcast(words & jnp.int32(-65536), F32).astype(BF16)

        def tmax(t):
            n = t.shape[1] // 128
            parts = [t[:, i * 128:(i + 1) * 128] for i in range(n)]
            while len(parts) > 1:
                parts = [jnp.maximum(parts[i], parts[i + 1]) if i + 1 < len(parts) else parts[i]
                         for i in range(0, len(parts), 2)]
            return parts[0]

        def tsum(t):
            n = t.shape[1] // 128
            parts = [t[:, i * 128:(i + 1) * 128] for i in range(n)]
            while len(parts) > 1:
                parts = [parts[i] + parts[i + 1] if i + 1 < len(parts) else parts[i]
                         for i in range(0, len(parts), 2)]
            return parts[0]

        def tie(p, lsum):
            n = p.shape[1] - 128
            last = jnp.minimum(p[:, n:], lsum)
            return last if n == 0 else jnp.concatenate([p[:, :n], last], axis=1)

        def attend(bufs, hh, hcol, qbs, TIE):
            q_s, kt_s, v_s = bufs
            cs = slice(hh * 128, (hh + 1) * 128)
            nsub = QB // 128
            for qb in qbs:
                r0 = qb * QB
                so = SOFF[qb]
                mx = None
                for c in range(qb):
                    st = _dot(q_s[pl.ds(r0, QB), cs], kt_s[cs, pl.ds(c * QB, QB)])
                    s_s[:, pl.ds(so + c * QB, QB)] = st
                    mx = tmax(st) if mx is None else jnp.maximum(mx, tmax(st))
                ms = []
                for a in range(nsub):
                    w = (a + 1) * 128
                    st = _dot(q_s[pl.ds(r0 + a * 128, 128), cs], kt_s[cs, pl.ds(r0, w)])
                    last = jnp.where(tri, st[:, a * 128:], -1e9)
                    st = last if a == 0 else jnp.concatenate([st[:, :a * 128], last], axis=1)
                    s_s[pl.ds(a * 128, 128), pl.ds(so + r0, w)] = st
                    ma = tmax(st)
                    if mx is not None:
                        ma = jnp.maximum(ma, mx[a * 128:(a + 1) * 128])
                    ms.append(jnp.broadcast_to(jnp.max(ma, axis=1, keepdims=True), (128, 128)))
                m = jnp.concatenate(ms, axis=0)
                lacc = None
                acc = None
                for c in range(qb):
                    p = jnp.exp2(s_s[:, pl.ds(so + c * QB, QB)] - jnp.concatenate([m] * nsub, axis=1))
                    lacc = tsum(p) if lacc is None else lacc + tsum(p)
                    pv = _dot((tie(p, lacc) if TIE else p).astype(BF16), v_s[pl.ds(c * QB, QB), cs])
                    acc = pv if acc is None else acc + pv
                for a in range(nsub):
                    w = (a + 1) * 128
                    p = jnp.exp2(s_s[pl.ds(a * 128, 128), pl.ds(so + r0, w)]
                                 - jnp.concatenate([ms[a]] * (a + 1), axis=1))
                    la = tsum(p)
                    if acc is not None:
                        la = la + lacc[a * 128:(a + 1) * 128]
                    pv = _dot((tie(p, la) if TIE else p).astype(BF16), v_s[pl.ds(r0, w), cs])
                    if acc is not None:
                        pv = pv + acc[a * 128:(a + 1) * 128]
                    l = jnp.broadcast_to(jnp.sum(la, axis=1, keepdims=True), (128, 128))
                    ctx_s[pl.ds(r0 + a * 128, 128), pl.ds(hcol, 128)] = (
                        pv * (g_s[pl.ds(r0 + a * 128, 128), :] * _rcp(l))).astype(BF16)

        def proj(hp, bufs, parts="qkv"):
            q_s, kt_s, v_s = bufs
            if "k" in parts:
                gather(wk_s, DC, hp, w2k_s)
                kt_s[...] = _dot(c_s[...], w2k_s[...]).astype(BF16).T
            if "q" in parts:
                gather(wq_s, M, hp, w2q_s)
                q_s[...] = (_dot(x_s[...], w2q_s[...]) * sc_a).astype(BF16)
            if "v" in parts:
                gather(wv_s, DC, hp, w2v_s)
                v_s[...] = _dot(c_s[...], w2v_s[...]).astype(BF16)

        def attn_proj(hp, bufs, hpn, bufsn, tie_rows=False):
            for item in PLAN:
                if isinstance(item, str):
                    if hpn is not None:
                        proj(hpn, bufsn, item)
                else:
                    hh, qb = item
                    attend(bufs, hh, pl.multiple_of(hp * 256 + hh * 128, 128), [qb], tie_rows)

        buf = ((q0_s, kt0_s, v0_s), (q1_s, kt1_s, v1_s))
        proj(0, buf[0])

        def a_body(i, carry):
            attn_proj(2 * i, buf[0], 2 * i + 1, buf[1])
            attn_proj(2 * i + 1, buf[1], 2 * i + 2, buf[0])
            return i + 1

        with jax.named_scope("abranch"):
            il = lax.fori_loop(0, H // 4 - 1, a_body, 0)
        cps[4].wait()
        cps[5].wait()
        with jax.named_scope("tail"):
            attn_proj(2 * il, buf[0], 2 * il + 1, buf[1], True)
            attn_proj(2 * il + 1, buf[1], None, None, True)

        @pl.when(il > 0)
        def _():
            final()

    pl.run_scoped(a_phase, pltpu.VMEM((QB, SOFF[S // QB]), F32))


@jax.jit
def pallas_gated_mix__compressed_kv_cla__sliding_local_dilated__prompt_kernel(
    A_x, A_c_kv, A_w_q, A_w_uk, A_w_uv, A_w_o, B_x, B_wqkv, B_wo, gate_w):
    del B_x
    any_spec = pl.BlockSpec(memory_space=pl.ANY)
    out = pl.pallas_call(
        _kernel,
        out_shape=jax.ShapeDtypeStruct((S, M), BF16),
        in_specs=[any_spec] * 8 + [pl.BlockSpec(memory_space=pltpu.VMEM)],
        out_specs=any_spec,
        scratch_shapes=[
            pltpu.VMEM((S, M), BF16),
            pltpu.VMEM((S, DC), BF16),
            pltpu.VMEM((M * 16, 128), jnp.int32),
            pltpu.VMEM((DC * 16, 128), jnp.int32),
            pltpu.VMEM((DC * 16, 128), jnp.int32),
            pltpu.VMEM((H * D + M, M), BF16),
            pltpu.VMEM((S, H * D + M), BF16),
            pltpu.VMEM((S, 128), F32),
            pltpu.VMEM((M, 256), BF16),
            pltpu.VMEM((DC, 256), BF16),
            pltpu.VMEM((DC, 256), BF16),
            pltpu.VMEM((S, 256), BF16),
            pltpu.VMEM((256, S), BF16),
            pltpu.VMEM((S, 256), BF16),
            pltpu.VMEM((S, 256), BF16),
            pltpu.VMEM((256, S), BF16),
            pltpu.VMEM((S, 256), BF16),
            pltpu.SemaphoreType.DMA((6 + S // RB + 4,)),
            pltpu.SemaphoreType.DMA((S // RF,)),
        ],
        compiler_params=pltpu.CompilerParams(vmem_limit_bytes=120 * 1024 * 1024),
    )(A_x.reshape(S, M), A_c_kv.reshape(S, DC), A_w_q.reshape(M * H, D), A_w_uk.reshape(DC * H, D),
      A_w_uv.reshape(DC * H, D), A_w_o.reshape(H * D, M), B_wqkv, B_wo, gate_w.reshape(1, M))
    return out.reshape(1, S, M)
```
